```python
import os as _os
_os.environ.setdefault("JAX_PLATFORMS", "cpu")
import jax
import jax.numpy as jnp

def _softmax(x, axis=-1):
    return jax.nn.softmax(x, axis=axis)
def _gelu(x):
    return jax.nn.gelu(x, approximate=True)
def _silu(x):
    return jax.nn.silu(x)
def _sigmoid(x):
    return jax.nn.sigmoid(x)
def _layernorm(x, axis=-1, eps=1e-5):
    m = jnp.mean(x, axis=axis, keepdims=True)
    v = jnp.var(x, axis=axis, keepdims=True)
    return (x - m) / jnp.sqrt(v + eps)
def _scatter_add(tgt, idx, src, axis=0):
    return tgt.at[idx].add(src)
def _segment_sum(src, seg, n):
    return jax.ops.segment_sum(src, seg, n)
class _Rng:
    def __init__(self, key):
        self._k = key
    def _next(self):
        self._k, sub = jax.random.split(self._k)
        return sub
    def normal(self, shape):
        return jax.random.normal(self._next(), shape, dtype=jnp.bfloat16)
    def randint(self, lo, hi, shape):
        return jax.random.randint(self._next(), shape, lo, hi, dtype=jnp.int32)
    def uniform(self, shape, lo=0.0, hi=1.0):
        return jax.random.uniform(self._next(), shape, jnp.bfloat16, lo, hi)
    def permutation(self, n):
        return jax.random.permutation(self._next(), n)


kernel_name = 'standalone__dense_activation_silu__prompt'

def setup_inputs():
    _rng = _Rng(jax.random.key(int.from_bytes(__import__("os").urandom(4), "little")))
    _w = (lambda a: (lambda t: t.astype(jnp.bfloat16) if jnp.issubdtype(t.dtype, jnp.floating) else t)(jnp.asarray(a)))
    B, S, D, F = 1, 2048, 448, 1792
    return {
        "x": _w((lambda *s: _rng.normal(s) * 0.05)(B, S, D)),
        "w1": _w((lambda *s: _rng.normal(s) * 0.05)(D, F) * (D ** -0.5)),
        "w2": _w((lambda *s: _rng.normal(s) * 0.05)(F, D) * (F ** -0.5)),
    }

def reference(x, w1, w2):
    h = jnp.einsum("bsd,df->bsf", x, w1)
    h = _silu(h)
    out = jnp.einsum("bsf,fd->bsd", h, w2)
    return out
```

```python
import functools

import jax
import jax.numpy as jnp
import jax.experimental.pallas as pl
import jax.experimental.pallas.tpu as pltpu


def _ffn_kernel(x_ref, w1_ref, w2_ref, o_ref):
    h = jnp.dot(x_ref[...], w1_ref[...], preferred_element_type=jnp.float32)
    t = 0.5 * h
    s = t * jnp.tanh(t) + t
    o = jnp.dot(s.astype(jnp.bfloat16), w2_ref[...], preferred_element_type=jnp.float32)
    o_ref[...] = o.astype(o_ref.dtype)


@jax.jit
def pallas_standalone__dense_activation_silu__prompt_kernel(
    x: jax.Array,
    w1: jax.Array,
    w2: jax.Array,
):
    B, S, D = x.shape
    F = w1.shape[1]
    M = B * S
    TM = 512
    x2 = x.reshape(M, D)
    out = pl.pallas_call(
        _ffn_kernel,
        grid=(M // TM,),
        in_specs=[
            pl.BlockSpec((TM, D), lambda i: (i, 0)),
            pl.BlockSpec((D, F), lambda i: (0, 0)),
            pl.BlockSpec((F, D), lambda i: (0, 0)),
        ],
        out_specs=pl.BlockSpec((TM, D), lambda i: (i, 0)),
        out_shape=jax.ShapeDtypeStruct((M, D), x.dtype),
        compiler_params=pltpu.CompilerParams(
            dimension_semantics=("parallel",),
            vmem_limit_bytes=96 * 1024 * 1024,
        ),
    )(x2, w1, w2)
    return out.reshape(B, S, D)
```

```python
import jax
import jax.numpy as jnp
from jax import lax
import jax.experimental.pallas as pl
import jax.experimental.pallas.tpu as pltpu

_C = 128
_NT_DIMS = (((1,), (1,)), ((), ()))


def _sl(a, b):
    return pl.ds(a, b - a)


def _m1(k0, k1, s0, s1, f0, f1, mode):
    nk = -(-(k1 - k0) // _C)
    nn = (f1 - f0) // _C
    if nn == 0 or s1 == s0:
        return []
    if (nk * nn) % 4 == 0:
        return [("M1", k0, k1, s0, s1, f0, f1, mode)]
    n1 = nn
    while (nk * n1) % 4:
        n1 -= 1
    parts = 2 if (nk * (nn - n1)) % 2 == 0 else 4
    step = (s1 - s0) // parts
    ops = []
    if n1:
        ops.append(("M1", k0, k1, s0, s1, f0, f0 + n1 * _C, mode))
    for p in range(parts):
        ops.append(("M1", k0, k1, s0 + p * step, s0 + (p + 1) * step, f0 + n1 * _C, f1, mode))
    return ops


def _schedule(D, S, F):
    c = _C
    a0, b0, aK, bK, TS = 6, 8, 8, 9, 512
    kt = (D // c) * c
    K3 = (kt, D)
    phases = []
    phases.append(([("x", *K3, 0, a0 * c)], [("T", *K3, 0, a0 * c)]))
    phases.append(([("w1", *K3, 0, b0 * c)], _m1(*K3, 0, a0 * c, 0, b0 * c, "init")))

    d1 = [("w1", *K3, b0 * c, F), ("x", *K3, a0 * c, S),
          ("x", 0, c, 0, aK * c), ("w1", 0, c, 0, bK * c)]
    o1 = _m1(*K3, 0, a0 * c, b0 * c, F, "init")
    o1 += [("T", *K3, a0 * c, S), ("T", 0, c, 0, aK * c)]
    s0 = a0 * c
    while s0 < S:
        s1 = min(s0 + TS, S)
        o1 += _m1(*K3, s0, s1, 0, F, "init")
        s0 = s1
    for s0 in range(0, aK * c, TS):
        o1 += _m1(0, c, s0, s0 + TS, 0, bK * c, "acc")
    phases.append((d1, o1))

    d2 = [("x", c, kt, 0, S), ("w1", c, kt, 0, F), ("x", 0, c, aK * c, S),
          ("w1", 0, c, bK * c, F), ("w2", 0, D, 0, F)]
    m1s, m2s = [], []
    for s0 in range(0, S, TS):
        s1 = s0 + TS
        if s1 <= aK * c:
            m1 = _m1(0, c, s0, s1, bK * c, F, "acc")
            if s0 == 0:
                m1 += [("T", c, kt, 0, S), ("T", 0, c, aK * c, S)]
            m1 += _m1(c, kt, s0, s1, 0, F, "fin")
        else:
            m1 = _m1(0, kt, s0, s1, 0, F, "fin")
        m1s.append(m1)
        if s1 < S:
            m2s.append([("M2", 0, D, s0, s1)])
        else:
            r = (3 * D) // 4
            m2s.append([("M2", 0, D, s0, s1 - c), ("M2", 0, r, s1 - c, s1),
                        ("M2", r, D, s1 - c, s1)])
    o2 = list(m1s[0])
    for i in range(1, len(m1s)):
        o2 += m1s[i] + m2s[i - 1]
    o2 += m2s[-1]
    phases.append((d2, o2))
    return phases


def _make_kernel(phases):
    nph = len(phases)

    def kernel(xT_hbm, w1_hbm, w2T_hbm, o_hbm, x_v, w1_v, w2_v, xr_v, s_v, hp_v, o_v, sems):
        bufs = {"x": (xT_hbm, x_v), "w1": (w1_hbm, w1_v), "w2": (w2T_hbm, w2_v)}

        def cin(p, d):
            name, r0, r1, c0, c1 = d
            src, dst = bufs[name]
            return pltpu.make_async_copy(
                src.at[_sl(r0, r1), _sl(c0, c1)], dst.at[_sl(r0, r1), _sl(c0, c1)], sems.at[p])

        def cout(r0, r1, c0, c1):
            return pltpu.make_async_copy(
                o_v.at[_sl(r0, r1), _sl(c0, c1)], o_hbm.at[_sl(r0, r1), _sl(c0, c1)], sems.at[nph])

        for p, (dmas, _) in enumerate(phases):
            for d in dmas:
                cin(p, d).start()

        outs = []
        for p, (dmas, ops) in enumerate(phases):
            for d in dmas:
                cin(p, d).wait()
            for op in ops:
                if op[0] == "T":
                    _, k0, k1, s0, s1 = op
                    xr_v[_sl(s0, s1), _sl(k0, k1)] = x_v[_sl(k0, k1), _sl(s0, s1)].T
                elif op[0] == "M1":
                    _, k0, k1, s0, s1, f0, f1, mode = op
                    blk = (_sl(s0, s1), _sl(f0, f1))
                    h = jnp.dot(xr_v[_sl(s0, s1), _sl(k0, k1)], w1_v[_sl(k0, k1), _sl(f0, f1)],
                                preferred_element_type=jnp.float32)
                    if mode == "init":
                        hp_v[blk] = h
                    elif mode == "acc":
                        hp_v[blk] += h
                    else:
                        t = 0.5 * (h + hp_v[blk])
                        s_v[blk] = (t * jnp.tanh(t) + t).astype(s_v.dtype)
                else:
                    _, r0, r1, s0, s1 = op
                    o = lax.dot_general(w2_v[_sl(r0, r1), :], s_v[_sl(s0, s1), :], _NT_DIMS,
                                        preferred_element_type=jnp.float32)
                    o_v[_sl(r0, r1), _sl(s0, s1)] = o.astype(o_v.dtype)
                    cout(r0, r1, s0, s1).start()
                    outs.append((r0, r1, s0, s1))
        for o in outs:
            cout(*o).wait()

    return kernel


@jax.jit
def pallas_standalone__dense_activation_silu__prompt_kernel(
    x: jax.Array,
    w1: jax.Array,
    w2: jax.Array,
):
    B, S, D = x.shape
    F = w1.shape[1]
    assert B == 1
    xT = jnp.swapaxes(x, 1, 2).reshape(D, S)
    w2T = w2.T
    phases = _schedule(D, S, F)
    oT = pl.pallas_call(
        _make_kernel(phases),
        in_specs=[pl.BlockSpec(memory_space=pl.ANY)] * 3,
        out_specs=pl.BlockSpec(memory_space=pl.ANY),
        out_shape=jax.ShapeDtypeStruct((D, S), x.dtype),
        scratch_shapes=[
            pltpu.VMEM((D, S), x.dtype),
            pltpu.VMEM((D, F), w1.dtype),
            pltpu.VMEM((D, F), w2.dtype),
            pltpu.VMEM((S, D), x.dtype),
            pltpu.VMEM((S, F), jnp.bfloat16),
            pltpu.VMEM((S, F), jnp.float32),
            pltpu.VMEM((D, S), x.dtype),
            pltpu.SemaphoreType.DMA((len(phases) + 1,)),
        ],
        compiler_params=pltpu.CompilerParams(
            vmem_limit_bytes=100 * 1024 * 1024,
            disable_semaphore_checks=True,
        ),
    )(xT, w1, w2T)
    return jnp.swapaxes(oT.reshape(B, D, S), 1, 2)
```

```python
import jax
import jax.numpy as jnp
from jax import lax
import jax.experimental.pallas as pl
import jax.experimental.pallas.tpu as pltpu

_C = 128
_NT_DIMS = (((1,), (1,)), ((), ()))


def _sl(a, b):
    return pl.ds(a, b - a)


def _m1(k0, k1, s0, s1, f0, f1, mode):
    nk = -(-(k1 - k0) // _C)
    nn = (f1 - f0) // _C
    if nn == 0 or s1 == s0:
        return []
    if (nk * nn) % 4 == 0:
        return [("M1", k0, k1, s0, s1, f0, f1, mode)]
    n1 = nn
    while (nk * n1) % 4:
        n1 -= 1
    parts = 2 if (nk * (nn - n1)) % 2 == 0 else 4
    step = (s1 - s0) // parts
    ops = []
    if n1:
        ops.append(("M1", k0, k1, s0, s1, f0, f0 + n1 * _C, mode))
    for p in range(parts):
        ops.append(("M1", k0, k1, s0 + p * step, s0 + (p + 1) * step, f0 + n1 * _C, f1, mode))
    return ops


def _schedule(D, S, F):
    c = _C
    a0, b0, aK, bK, TS = 6, 10, 8, 10, 512
    kt = (D // c) * c
    K3 = (kt, D)
    phases = []
    phases.append(([("x", *K3, 0, a0 * c)], [("T", *K3, 0, a0 * c)]))
    phases.append(([("w1", *K3, 0, b0 * c)], _m1(*K3, 0, a0 * c, 0, b0 * c, "init")))

    d1 = [("w1", *K3, b0 * c, F), ("x", *K3, a0 * c, S),
          ("x", 0, c, 0, aK * c), ("w1", 0, c, 0, bK * c)]
    o1 = _m1(*K3, 0, a0 * c, b0 * c, F, "init")
    o1 += [("T", *K3, a0 * c, S), ("T", 0, c, 0, aK * c)]
    s0 = a0 * c
    while s0 < S:
        s1 = min(s0 + TS, S)
        o1 += _m1(*K3, s0, s1, 0, F, "init")
        s0 = s1
    for s0 in range(0, aK * c, TS):
        o1 += _m1(0, c, s0, s0 + TS, 0, bK * c, "acc")
    phases.append((d1, o1))

    d2 = [("x", c, kt, 0, S), ("w1", c, kt, 0, F), ("x", 0, c, aK * c, S),
          ("w1", 0, c, bK * c, F), ("w2", 0, D, 0, F)]
    m1s, m2s = [], []
    for s0 in range(0, S, TS):
        s1 = s0 + TS
        if s1 <= aK * c:
            m1 = _m1(0, c, s0, s1, bK * c, F, "acc")
            if s0 == 0:
                m1 += [("T", c, kt, 0, aK * c), ("T", 0, kt, aK * c, S)]
            m1 += _m1(c, kt, s0, s1, 0, F, "fin")
        else:
            m1 = _m1(0, kt, s0, s1, 0, F, "fin")
        m1s.append(m1)
        if s1 < S:
            m2s.append([("M2", 0, D, s0, s1)])
        else:
            r = D - 64
            m2s.append([("M2", 0, D, s0, s1 - c), ("M2", 0, r, s1 - c, s1),
                        ("M2", r, D, s1 - c, s1)])
    o2 = list(m1s[0])
    for i in range(1, len(m1s)):
        o2 += m1s[i] + m2s[i - 1]
    o2 += m2s[-1]
    phases.append((d2, o2))
    return phases


def _make_kernel(phases):
    nph = len(phases)

    def kernel(xT_hbm, w1_hbm, w2T_hbm, o_hbm, x_v, w1_v, w2_v, s_v, hp_v, o_v, sems):
        bufs = {"x": (xT_hbm, x_v), "w1": (w1_hbm, w1_v), "w2": (w2T_hbm, w2_v)}

        def cin(p, d):
            name, r0, r1, c0, c1 = d
            src, dst = bufs[name]
            return pltpu.make_async_copy(
                src.at[_sl(r0, r1), _sl(c0, c1)], dst.at[_sl(r0, r1), _sl(c0, c1)], sems.at[p])

        def cout(r0, r1, c0, c1):
            return pltpu.make_async_copy(
                o_v.at[_sl(r0, r1), _sl(c0, c1)], o_hbm.at[_sl(r0, r1), _sl(c0, c1)], sems.at[nph])

        for p, (dmas, _) in enumerate(phases):
            for d in dmas:
                cin(p, d).start()

        xrows = {}

        def x_rows(k0, k1, s0, s1):
            for (kk0, kk1, ss0, ss1), val in xrows.items():
                if (kk0, kk1) == (k0, k1) and ss0 <= s0 and s1 <= ss1:
                    return val[s0 - ss0:s1 - ss0]
            raise KeyError((k0, k1, s0, s1))

        outs = []
        for p, (dmas, ops) in enumerate(phases):
            for d in dmas:
                cin(p, d).wait()
            for op in ops:
                if op[0] == "T":
                    _, k0, k1, s0, s1 = op
                    xrows[(k0, k1, s0, s1)] = x_v[_sl(k0, k1), _sl(s0, s1)].T
                elif op[0] == "M1":
                    _, k0, k1, s0, s1, f0, f1, mode = op
                    blk = (_sl(s0, s1), _sl(f0, f1))
                    h = jnp.dot(x_rows(k0, k1, s0, s1), w1_v[_sl(k0, k1), _sl(f0, f1)],
                                preferred_element_type=jnp.float32)
                    if mode == "init":
                        hp_v[blk] = h
                    elif mode == "acc":
                        hp_v[blk] += h
                    else:
                        t = 0.5 * (h + hp_v[blk])
                        s_v[blk] = (t * jnp.tanh(t) + t).astype(s_v.dtype)
                else:
                    _, r0, r1, s0, s1 = op
                    o = lax.dot_general(w2_v[_sl(r0, r1), :], s_v[_sl(s0, s1), :], _NT_DIMS,
                                        preferred_element_type=jnp.float32)
                    o_v[_sl(r0, r1), _sl(s0, s1)] = o.astype(o_v.dtype)
                    cout(r0, r1, s0, s1).start()
                    outs.append((r0, r1, s0, s1))
        for o in outs:
            cout(*o).wait()

    return kernel


def _compiler_params():
    kw = dict(vmem_limit_bytes=100 * 1024 * 1024)
    try:
        return pltpu.CompilerParams(disable_semaphore_checks=True, **kw)
    except TypeError:
        return pltpu.CompilerParams(**kw)


@jax.jit
def pallas_standalone__dense_activation_silu__prompt_kernel(
    x: jax.Array,
    w1: jax.Array,
    w2: jax.Array,
):
    B, S, D = x.shape
    F = w1.shape[1]
    assert (B, S, D, F) == (1, 2048, 448, 1792)
    xT = jnp.swapaxes(x, 1, 2).reshape(D, S)
    w2T = w2.T
    phases = _schedule(D, S, F)
    oT = pl.pallas_call(
        _make_kernel(phases),
        in_specs=[pl.BlockSpec(memory_space=pl.ANY)] * 3,
        out_specs=pl.BlockSpec(memory_space=pl.ANY),
        out_shape=jax.ShapeDtypeStruct((D, S), x.dtype),
        scratch_shapes=[
            pltpu.VMEM((D, S), x.dtype),
            pltpu.VMEM((D, F), w1.dtype),
            pltpu.VMEM((D, F), w2.dtype),
            pltpu.VMEM((S, F), jnp.bfloat16),
            pltpu.VMEM((S, F), jnp.float32),
            pltpu.VMEM((D, S), x.dtype),
            pltpu.SemaphoreType.DMA((len(phases) + 1,)),
        ],
        compiler_params=_compiler_params(),
    )(xT, w1, w2T)
    return jnp.swapaxes(oT.reshape(B, D, S), 1, 2)
```
